```python
import jax
import jax.numpy as jnp

def _softmax(x, axis=-1):
    return jax.nn.softmax(x, axis=axis)
def _gelu(x):
    return jax.nn.gelu(x, approximate=True)
def _silu(x):
    return jax.nn.silu(x)
def _sigmoid(x):
    return jax.nn.sigmoid(x)
def _layernorm(x, axis=-1, eps=1e-5):
    m = jnp.mean(x, axis=axis, keepdims=True)
    v = jnp.var(x, axis=axis, keepdims=True)
    return (x - m) / jnp.sqrt(v + eps)
def _scatter_add(tgt, idx, src, axis=0):
    return tgt.at[idx].add(src)
def _segment_sum(src, seg, n):
    return jax.ops.segment_sum(src, seg, n)
class _Rng:
    def __init__(self, key):
        self._k = key
    def _next(self):
        self._k, sub = jax.random.split(self._k)
        return sub
    def normal(self, shape):
        return jax.random.normal(self._next(), shape, dtype=jnp.bfloat16)
    def randint(self, lo, hi, shape):
        return jax.random.randint(self._next(), shape, lo, hi, dtype=jnp.int32)
    def uniform(self, shape, lo=0.0, hi=1.0):
        return jax.random.uniform(self._next(), shape, jnp.bfloat16, lo, hi)
    def permutation(self, n):
        return jax.random.permutation(self._next(), n)


kernel_name = 'gated_mix__sliding_local_dilated__glu_gated_reglu__prompt'

def setup_inputs():
    _rng = _Rng(jax.random.key(int.from_bytes(__import__("os").urandom(4), "little")))
    _w = (lambda a: (lambda t: t.astype(jnp.bfloat16) if jnp.issubdtype(t.dtype, jnp.floating) else t)(jnp.asarray(a)))
    def _A_setup():
        B, S, D = 1, 2048, 1024
        return {
            "x": _w((lambda *s: _rng.normal(s) * 0.05)(B, S, D)),
            "wqkv": _w((lambda *s: _rng.normal(s) * 0.05)(D, 3 * D)),
            "wo": _w((lambda *s: _rng.normal(s) * 0.05)(D, D)),
        }
    _A_in = _A_setup()

    def _B_setup():
        B, S, D, F = 1, 2048, 1024, 3584
        return {
            "x": _w((lambda *s: _rng.normal(s) * 0.05)(B, S, D)),
            "W_gate": _w((lambda *s: _rng.normal(s) * 0.05)(D, F) * (2.0 / D) ** 0.5),
            "W_up": _w((lambda *s: _rng.normal(s) * 0.05)(D, F) * (2.0 / D) ** 0.5),
            "W_down": _w((lambda *s: _rng.normal(s) * 0.05)(F, D) * (1.0 / F) ** 0.5),
        }
    _B_in = _B_setup()

    return {
        "A_x": _A_in["x"],
        "A_wqkv": _A_in["wqkv"],
        "A_wo": _A_in["wo"],
        "B_x": _B_in["x"],
        "B_W_gate": _B_in["W_gate"],
        "B_W_up": _B_in["W_up"],
        "B_W_down": _B_in["W_down"],
        "gate_w": _w((lambda *s: _rng.normal(s) * 0.05)(1024)),
    }

def reference(A_x, A_wqkv, A_wo, B_x, B_W_gate, B_W_up, B_W_down, gate_w):
    def _A_ref(x, wqkv, wo):
        B, S, D = x.shape
        H = 32; Dh = D // H
        W, dil = 8, 2
        qkv = (lambda x, *d: x.transpose(*d))((x @ wqkv).reshape(B, S, 3, H, Dh), 2, 0, 3, 1, 4)
        q, k, v = qkv[0], qkv[1], qkv[2]
        scale = Dh ** -0.5
        pos = jnp.arange(S)
        off = jnp.arange(W) * dil
        idx = pos[:, None] - off[None, :]
        mask = idx >= 0
        idx_c = jnp.where(mask, idx, 0).reshape(-1)
        kg = k[:, :, idx_c, :].reshape(B, H, S, W, Dh)
        vg = v[:, :, idx_c, :].reshape(B, H, S, W, Dh)
        logits = jnp.einsum("bhsd,bhswd->bhsw", q, kg) * scale
        logits = jnp.where(mask[None, None, :, :], logits, -1e9)
        attn = _softmax(logits, axis=-1)
        o = jnp.einsum("bhsw,bhswd->bhsd", attn, vg)
        return (lambda x, *d: x.transpose(*d))(o, 0, 2, 1, 3).reshape(B, S, D) @ wo

    def _B_ref(x, W_gate, W_up, W_down):
        gate = jnp.einsum("bsd,df->bsf", x, W_gate)
        up = jnp.einsum("bsd,df->bsf", x, W_up)
        gate = gate * (lambda x, dt: x.astype(dt))(gate > 0, gate.dtype)
        h = gate * up
        return jnp.einsum("bsf,fd->bsd", h, W_down)

    x = A_x
    g = _sigmoid((x * gate_w).sum(-1, keepdims=True))
    a = _A_ref(x, A_wqkv, A_wo)
    b = _B_ref(x, B_W_gate, B_W_up, B_W_down)
    return g * a + (1 - g) * b
```

```python
import functools

import jax
import jax.numpy as jnp
import jax.experimental.pallas as pl
import jax.experimental.pallas.tpu as pltpu

_TM = 512
_TF = 512
_R = 16
_HALO = 16
_H, _W, _DIL = 32, 8, 2
_NEG = -1e9


def _dot(a, b):
    return jnp.dot(a, b, preferred_element_type=jnp.float32)


def _butterfly(chunks, lane):
    chunks = list(chunks)
    for cbit, lbit in ((4, 16), (2, 8), (1, 4)):
        low = (lane & lbit) == 0
        for c in range(8):
            if c & cbit:
                continue
            a, b = chunks[c], chunks[c | cbit]
            chunks[c] = jnp.where(low, a, pltpu.roll(b, lbit, 1))
            chunks[c | cbit] = jnp.where(low, pltpu.roll(a, 128 - lbit, 1), b)
    return chunks


def _allreduce4(x, lane):
    for bit in (1, 2):
        low = (lane & bit) == 0
        x = x + jnp.where(low, pltpu.roll(x, 128 - bit, 1), pltpu.roll(x, bit, 1))
    return x


def _kernel(x_ref, gw_ref, wqkv_hbm, wo_hbm, wg_hbm, wu_hbm, wd_hbm, o_ref,
            wqkv, wo, wg, wu, wd, qbuf, kbuf, vbuf, obuf, hbuf, sems):
    tm, D = x_ref.shape
    F = wg.shape[1]
    tf = _TF
    nf = F // tf
    step = pl.program_id(0)
    scale = (D // _H) ** -0.5

    def cp_qkv(p):
        return pltpu.make_async_copy(wqkv_hbm.at[:, pl.ds(p * D, D)],
                                     wqkv.at[:, pl.ds(p * D, D)], sems.at[p])

    def cp_g(j):
        return pltpu.make_async_copy(wg_hbm.at[:, pl.ds(j * tf, tf)],
                                     wg.at[:, pl.ds(j * tf, tf)], sems.at[3 + j])

    def cp_u(j):
        return pltpu.make_async_copy(wu_hbm.at[:, pl.ds(j * tf, tf)],
                                     wu.at[:, pl.ds(j * tf, tf)], sems.at[3 + nf + j])

    def cp_d():
        return pltpu.make_async_copy(wd_hbm, wd, sems.at[3 + 2 * nf])

    def cp_o():
        return pltpu.make_async_copy(wo_hbm, wo, sems.at[4 + 2 * nf])

    def attention(r0, first):
        lane = jax.lax.broadcasted_iota(jnp.int32, (_R, 128), 1)
        q = [qbuf[pl.ds(r0, _R), pl.ds(c * 128, 128)] for c in range(8)]
        logits = []
        for w in range(_W):
            base = _HALO + r0 - _DIL * w
            acc = q[0] * kbuf[pl.ds(base, _R), pl.ds(0, 128)]
            for c in range(1, 8):
                acc = acc + q[c] * kbuf[pl.ds(base, _R), pl.ds(c * 128, 128)]
            l = _allreduce4(acc, lane) * scale
            if first and r0 < _DIL * w:
                row = jax.lax.broadcasted_iota(jnp.int32, (_R, 128), 0) + r0
                l = jnp.where(row >= _DIL * w, l, _NEG)
            logits.append(l)
        m = logits[0]
        for l in logits[1:]:
            m = jnp.maximum(m, l)
        e = [jnp.exp(l - m) for l in logits]
        s = e[0]
        for t in e[1:]:
            s = s + t
        inv = 1.0 / s
        p = [t * inv for t in e]
        outs = []
        for c in range(8):
            acc = p[0] * vbuf[pl.ds(_HALO + r0, _R), pl.ds(c * 128, 128)]
            for w in range(1, _W):
                base = _HALO + r0 - _DIL * w
                acc = acc + p[w] * vbuf[pl.ds(base, _R), pl.ds(c * 128, 128)]
            outs.append(acc)
        outs = _butterfly(outs, lane)
        for c in range(8):
            obuf[pl.ds(r0, _R), pl.ds(c * 128, 128)] = outs[c].astype(obuf.dtype)

    def project(p, dst, off):
        r = _dot(x_ref[...], wqkv[:, p * D:(p + 1) * D])
        r = r.astype(jnp.bfloat16).astype(jnp.float32)
        for r0 in range(0, tm, _R):
            lane = jax.lax.broadcasted_iota(jnp.int32, (_R, 128), 1)
            ch = [r[r0:r0 + _R, c * 128:(c + 1) * 128] for c in range(8)]
            ch = _butterfly(ch, lane)
            for c in range(8):
                dst[pl.ds(off + r0, _R), pl.ds(c * 128, 128)] = ch[c]

    def body(first):
        if first:
            for p in (1, 2, 0):
                cp_qkv(p).start()
            for j in range(nf):
                cp_g(j).start()
                cp_u(j).start()
            cp_d().start()
            cp_o().start()
        else:
            kbuf[pl.ds(0, _HALO), :] = kbuf[pl.ds(tm, _HALO), :]
            vbuf[pl.ds(0, _HALO), :] = vbuf[pl.ds(tm, _HALO), :]
        for p, dst, off in ((1, kbuf, _HALO), (2, vbuf, _HALO), (0, qbuf, 0)):
            if first:
                cp_qkv(p).wait()
            project(p, dst, off)
        if first:
            kbuf[pl.ds(0, _HALO), :] = jnp.zeros((_HALO, D), jnp.float32)
            vbuf[pl.ds(0, _HALO), :] = jnp.broadcast_to(
                vbuf[pl.ds(_HALO, 1), :], (_HALO, D))

        nblk = tm // _R
        for j in range(nf):
            if first:
                cp_g(j).wait()
                cp_u(j).wait()
            g = _dot(x_ref[...], wg[:, j * tf:(j + 1) * tf])
            u = _dot(x_ref[...], wu[:, j * tf:(j + 1) * tf])
            g = g.astype(jnp.bfloat16).astype(jnp.float32)
            u = u.astype(jnp.bfloat16).astype(jnp.float32)
            g = g * (g > 0).astype(jnp.float32)
            hbuf[:, j * tf:(j + 1) * tf] = (g * u).astype(hbuf.dtype)
            for b in range(j * nblk // nf, (j + 1) * nblk // nf):
                attention(b * _R, first)
        if first:
            cp_d().wait()
        b_out = _dot(hbuf[...], wd[...])
        if first:
            cp_o().wait()
        a_out = _dot(obuf[...], wo[...])
        xg = (x_ref[...] * gw_ref[...]).astype(jnp.float32)
        gate = jax.nn.sigmoid(jnp.sum(xg, axis=-1, keepdims=True))
        o_ref[...] = (gate * a_out + (1.0 - gate) * b_out).astype(o_ref.dtype)

    @pl.when(step == 0)
    def _():
        body(True)

    @pl.when(step > 0)
    def _():
        body(False)


@jax.jit
def pallas_gated_mix__sliding_local_dilated__glu_gated_reglu__prompt_kernel(
    A_x: jax.Array,
    A_wqkv: jax.Array,
    A_wo: jax.Array,
    B_x: jax.Array,
    B_W_gate: jax.Array,
    B_W_up: jax.Array,
    B_W_down: jax.Array,
    gate_w: jax.Array,
):
    del B_x
    B, S, D = A_x.shape
    F = B_W_gate.shape[1]
    assert B == 1
    tm = _TM
    nf = F // _TF
    dt = A_x.dtype
    hbm = pl.BlockSpec(memory_space=pl.ANY)
    out = pl.pallas_call(
        _kernel,
        grid=(S // tm,),
        in_specs=[
            pl.BlockSpec((tm, D), lambda i: (i, 0)),
            pl.BlockSpec((1, D), lambda i: (0, 0)),
            hbm, hbm, hbm, hbm, hbm,
        ],
        out_specs=pl.BlockSpec((tm, D), lambda i: (i, 0)),
        out_shape=jax.ShapeDtypeStruct((S, D), dt),
        scratch_shapes=[
            pltpu.VMEM((D, 3 * D), dt),
            pltpu.VMEM((D, D), dt),
            pltpu.VMEM((D, F), dt),
            pltpu.VMEM((D, F), dt),
            pltpu.VMEM((F, D), dt),
            pltpu.VMEM((tm, D), jnp.float32),
            pltpu.VMEM((_HALO + tm, D), jnp.float32),
            pltpu.VMEM((_HALO + tm, D), jnp.float32),
            pltpu.VMEM((tm, D), dt),
            pltpu.VMEM((tm, F), dt),
            pltpu.SemaphoreType.DMA((5 + 2 * nf,)),
        ],
        compiler_params=pltpu.CompilerParams(
            dimension_semantics=("arbitrary",),
            vmem_limit_bytes=100 * 1024 * 1024,
        ),
    )(A_x.reshape(S, D), gate_w.reshape(1, D), A_wqkv, A_wo, B_W_gate, B_W_up, B_W_down)
    return out.reshape(B, S, D)
```

```python
import jax
import jax.numpy as jnp
import jax.experimental.pallas as pl
import jax.experimental.pallas.tpu as pltpu

_TN = 256
_TF = 512
_R = 16
_HALO = 16
_H, _W, _DIL = 32, 8, 2
_NEG = -1e9


def _dot(a, b):
    return jnp.dot(a, b, preferred_element_type=jnp.float32)


def _butterfly(chunks, lane):
    chunks = list(chunks)
    for cbit, lbit in ((4, 16), (2, 8), (1, 4)):
        low = (lane & lbit) == 0
        for c in range(8):
            if c & cbit:
                continue
            a, b = chunks[c], chunks[c | cbit]
            chunks[c] = jnp.where(low, a, pltpu.roll(b, lbit, 1))
            chunks[c | cbit] = jnp.where(low, pltpu.roll(a, 128 - lbit, 1), b)
    return chunks


def _allreduce4(x, lane):
    for bit in (1, 2):
        low = (lane & bit) == 0
        x = x + jnp.where(low, pltpu.roll(x, 128 - bit, 1), pltpu.roll(x, bit, 1))
    return x


def _kernel(gw_ref, x_hbm, wqkv_hbm, wo_hbm, wg_hbm, wu_hbm, wd_hbm, o_hbm,
            xb, wqkv, wo, wg, wu, wd, qbuf, kbuf, vbuf, obuf, hbuf, gbuf, outb,
            sem_x, sem_qkv, sem_g, sem_u, sem_do, sem_out):
    S, D = xb.shape
    F = wg.shape[1]
    tf = _TF
    nf = F // tf
    scale = (D // _H) ** -0.5

    def cp_x():
        return pltpu.make_async_copy(x_hbm, xb, sem_x)

    def cp_qkv(p):
        return pltpu.make_async_copy(wqkv_hbm.at[:, pl.ds(p * D, D)],
                                     wqkv.at[:, pl.ds(p * D, D)], sem_qkv.at[p])

    def cp_g(j):
        c = pl.ds(pl.multiple_of(j * tf, tf), tf)
        return pltpu.make_async_copy(wg_hbm.at[:, c], wg.at[:, c], sem_g.at[j])

    def cp_u(j):
        c = pl.ds(pl.multiple_of(j * tf, tf), tf)
        return pltpu.make_async_copy(wu_hbm.at[:, c], wu.at[:, c], sem_u.at[j])

    def cp_d():
        return pltpu.make_async_copy(wd_hbm, wd, sem_do.at[0])

    def cp_o():
        return pltpu.make_async_copy(wo_hbm, wo, sem_do.at[1])

    def cp_out(n):
        c = pl.ds(pl.multiple_of(n * _TN, _TN), _TN)
        return pltpu.make_async_copy(outb.at[:, c], o_hbm.at[:, c], sem_out.at[n])

    def attention(r0, first):
        lane = jax.lax.broadcasted_iota(jnp.int32, (_R, 128), 1)
        q = [qbuf[pl.ds(r0, _R), pl.ds(c * 128, 128)] for c in range(8)]
        accs = [None] * _W
        for c in range(8):
            win = kbuf[pl.ds(r0, _HALO + _R), pl.ds(c * 128, 128)]
            for w in range(_W):
                o = _HALO - _DIL * w
                t = q[c] * win[o:o + _R]
                accs[w] = t if c == 0 else accs[w] + t
        logits = []
        for w in range(_W):
            acc = accs[w]
            l = _allreduce4(acc, lane) * scale
            if first and _DIL * w > 0:
                row = jax.lax.broadcasted_iota(jnp.int32, (_R, 128), 0)
                l = jnp.where(row >= _DIL * w, l, _NEG)
            logits.append(l)
        m = logits[0]
        for l in logits[1:]:
            m = jnp.maximum(m, l)
        e = [jnp.exp(l - m) for l in logits]
        s = e[0]
        for t in e[1:]:
            s = s + t
        inv = 1.0 / s
        p = [t * inv for t in e]
        outs = []
        for c in range(8):
            win = vbuf[pl.ds(r0, _HALO + _R), pl.ds(c * 128, 128)]
            acc = p[0] * win[_HALO:]
            for w in range(1, _W):
                o = _HALO - _DIL * w
                acc = acc + p[w] * win[o:o + _R]
            outs.append(acc)
        outs = _butterfly(outs, lane)
        for c in range(8):
            obuf[pl.ds(r0, _R), pl.ds(c * 128, 128)] = outs[c].astype(obuf.dtype)

    def project(p, dst, off):
        r = _dot(xb[...], wqkv[:, p * D:(p + 1) * D])
        r = r.astype(jnp.bfloat16).astype(jnp.float32)
        lane = jax.lax.broadcasted_iota(jnp.int32, (_R, 128), 1)
        for r0 in range(0, S, _R):
            ch = [r[r0:r0 + _R, c * 128:(c + 1) * 128] for c in range(8)]
            ch = _butterfly(ch, lane)
            for c in range(8):
                dst[pl.ds(off + r0, _R), pl.ds(c * 128, 128)] = ch[c]

    cp_x().start()
    cp_qkv(1).start()
    cp_x().wait()
    cp_qkv(2).start()
    cp_qkv(1).wait()
    cp_qkv(0).start()
    for j in range(nf):
        cp_g(j).start()
        cp_u(j).start()
    cp_d().start()
    cp_o().start()

    project(1, kbuf, _HALO)
    cp_qkv(2).wait()
    project(2, vbuf, _HALO)
    cp_qkv(0).wait()
    project(0, qbuf, 0)
    kbuf[pl.ds(0, _HALO), :] = jnp.zeros((_HALO, D), jnp.float32)
    vbuf[pl.ds(0, _HALO), :] = jnp.broadcast_to(vbuf[pl.ds(_HALO, 1), :], (_HALO, D))
    attention(0, True)

    xg = (xb[...] * gw_ref[...].reshape(1, D)).astype(jnp.float32)
    gbuf[...] = jnp.broadcast_to(
        jax.nn.sigmoid(jnp.sum(xg, axis=-1, keepdims=True)), gbuf.shape)

    nblk = S // _R
    per = -(-(nblk - 1) // nf)

    def ffn(j):
        cp_g(j).wait()
        cp_u(j).wait()
        c = pl.ds(pl.multiple_of(j * tf, tf), tf)
        g = _dot(xb[...], wg[:, c])
        u = _dot(xb[...], wu[:, c])
        g = g.astype(jnp.bfloat16).astype(jnp.float32)
        u = u.astype(jnp.bfloat16).astype(jnp.float32)
        g = g * (g > 0).astype(jnp.float32)
        hbuf[:, c] = (g * u).astype(hbuf.dtype)
        b0 = jnp.minimum(1 + j * per, nblk - per)
        for b in range(per):
            attention(pl.multiple_of((b0 + b) * _R, _R), False)

    pl.loop(0, nf)(ffn)
    cp_d().wait()
    cp_o().wait()

    def final(n):
        c = pl.ds(pl.multiple_of(n * _TN, _TN), _TN)
        b_out = _dot(hbuf[...], wd[:, c])
        a_out = _dot(obuf[...], wo[:, c])
        gate = jnp.concatenate([gbuf[...]] * (_TN // 128), axis=1)
        outb[:, c] = (gate * a_out + (1.0 - gate) * b_out).astype(outb.dtype)
        cp_out(n).start()

    pl.loop(0, D // _TN)(final)
    for n in range(D // _TN):
        cp_out(n).wait()


@jax.jit
def pallas_gated_mix__sliding_local_dilated__glu_gated_reglu__prompt_kernel(
    A_x: jax.Array,
    A_wqkv: jax.Array,
    A_wo: jax.Array,
    B_x: jax.Array,
    B_W_gate: jax.Array,
    B_W_up: jax.Array,
    B_W_down: jax.Array,
    gate_w: jax.Array,
):
    del B_x
    B, S, D = A_x.shape
    F = B_W_gate.shape[1]
    assert B == 1
    nf = F // _TF
    dt = A_x.dtype
    hbm = pl.BlockSpec(memory_space=pl.ANY)
    out = pl.pallas_call(
        _kernel,
        in_specs=[pl.BlockSpec(memory_space=pltpu.VMEM)] + [hbm] * 6,
        out_specs=hbm,
        out_shape=jax.ShapeDtypeStruct((S, D), dt),
        scratch_shapes=[
            pltpu.VMEM((S, D), dt),
            pltpu.VMEM((D, 3 * D), dt),
            pltpu.VMEM((D, D), dt),
            pltpu.VMEM((D, F), dt),
            pltpu.VMEM((D, F), dt),
            pltpu.VMEM((F, D), dt),
            pltpu.VMEM((S, D), jnp.float32),
            pltpu.VMEM((_HALO + S, D), jnp.float32),
            pltpu.VMEM((_HALO + S, D), jnp.float32),
            pltpu.VMEM((S, D), dt),
            pltpu.VMEM((S, F), dt),
            pltpu.VMEM((S, 128), jnp.float32),
            pltpu.VMEM((S, D), dt),
            pltpu.SemaphoreType.DMA(()),
            pltpu.SemaphoreType.DMA((3,)),
            pltpu.SemaphoreType.DMA((nf,)),
            pltpu.SemaphoreType.DMA((nf,)),
            pltpu.SemaphoreType.DMA((2,)),
            pltpu.SemaphoreType.DMA((D // _TN,)),
        ],
        compiler_params=pltpu.CompilerParams(vmem_limit_bytes=124 * 1024 * 1024),
    )(gate_w, A_x.reshape(S, D), A_wqkv, A_wo, B_W_gate, B_W_up, B_W_down)
    return out.reshape(B, S, D)
```
